```python
import os as _os
_os.environ.setdefault("JAX_PLATFORMS", "cpu")
import jax
import jax.numpy as jnp

def _softmax(x, axis=-1):
    return jax.nn.softmax(x, axis=axis)
def _gelu(x):
    return jax.nn.gelu(x, approximate=True)
def _silu(x):
    return jax.nn.silu(x)
def _sigmoid(x):
    return jax.nn.sigmoid(x)
def _layernorm(x, axis=-1, eps=1e-5):
    m = jnp.mean(x, axis=axis, keepdims=True)
    v = jnp.var(x, axis=axis, keepdims=True)
    return (x - m) / jnp.sqrt(v + eps)
def _scatter_add(tgt, idx, src, axis=0):
    return tgt.at[idx].add(src)
def _segment_sum(src, seg, n):
    return jax.ops.segment_sum(src, seg, n)
class _Rng:
    def __init__(self, key):
        self._k = key
    def _next(self):
        self._k, sub = jax.random.split(self._k)
        return sub
    def normal(self, shape):
        return jax.random.normal(self._next(), shape, dtype=jnp.bfloat16)
    def randint(self, lo, hi, shape):
        return jax.random.randint(self._next(), shape, lo, hi, dtype=jnp.int32)
    def uniform(self, shape, lo=0.0, hi=1.0):
        return jax.random.uniform(self._next(), shape, jnp.bfloat16, lo, hi)
    def permutation(self, n):
        return jax.random.permutation(self._next(), n)


kernel_name = 'parallel_sum__sliding_block_cached__dense_activation_mish__decode'

def setup_inputs():
    _rng = _Rng(jax.random.key(int.from_bytes(__import__("os").urandom(4), "little")))
    _w = (lambda a: (lambda t: t.astype(jnp.bfloat16) if jnp.issubdtype(t.dtype, jnp.floating) else t)(jnp.asarray(a)))
    def _A_setup():
        B, Sq, D = 2, 1, 512
        Hq, Hkv, Sk, Dh = 32, 8, 32768, 128
        assert Hq % Hkv == 0, (Hq, Hkv)
        return {
            "x": _w((lambda *s: _rng.normal(s) * 0.05)(B, Sq, D)),
            "k_cache": _w((lambda *s: _rng.normal(s) * 0.8)(B, Hkv, Sk, Dh)),
            "v_cache": _w((lambda *s: _rng.normal(s) * 0.8)(B, Hkv, Sk, Dh)),
            "wq": _w((lambda *s: _rng.normal(s) * 0.8)(D, Hq * Dh) * (D ** -0.5)),
            "wo": _w((lambda *s: _rng.normal(s) * 0.8)(Hq * Dh, D) * ((Hq * Dh) ** -0.5)),
        }
    _A_in = _A_setup()

    def _B_setup():
        B, S, D, F = 2, 1, 512, 1792
        return {
            "x": _w((lambda *s: _rng.normal(s) * 0.05)(B, S, D)),
            "w1": _w((lambda *s: _rng.normal(s) * 0.4)(D, F) * (D ** -0.5)),
            "b1": _w((lambda *s: _rng.normal(s) * 0.05)(F)),
            "w2": _w((lambda *s: _rng.normal(s) * 0.05)(F, D) * (F ** -0.5)),
        }
    _B_in = _B_setup()

    return {
        "A_x": _A_in["x"],
        "A_k_cache": _A_in["k_cache"],
        "A_v_cache": _A_in["v_cache"],
        "A_wq": _A_in["wq"],
        "A_wo": _A_in["wo"],
        "B_x": _B_in["x"],
        "B_w1": _B_in["w1"],
        "B_b1": _B_in["b1"],
        "B_w2": _B_in["w2"],
    }

def reference(A_x, A_k_cache, A_v_cache, A_wq, A_wo, B_x, B_w1, B_b1, B_w2):
    def _A_ref(x, k_cache, v_cache, wq, wo):
        B, Sq, D = x.shape
        Hq, Dh = 32, 128
        Hkv, Sk = k_cache.shape[1], k_cache.shape[2]
        W = min(4096, max(256, Sk // 4))
        rep = Hq // Hkv
        q = (lambda x, *d: x.transpose(*d))((x @ wq).reshape(B, Sq, Hq, Dh), 0, 2, 1, 3)
        k = jnp.repeat(k_cache[:, :, Sk - W:, :], rep, axis=1)
        v = jnp.repeat(v_cache[:, :, Sk - W:, :], rep, axis=1)
        scores = jnp.einsum("bhqd,bhkd->bhqk", q, k) * (Dh ** -0.5)
        p = _softmax(scores, axis=-1)
        o = jnp.einsum("bhqk,bhkd->bhqd", p, v)
        return (lambda x, *d: x.transpose(*d))(o, 0, 2, 1, 3).reshape(B, Sq, Hq * Dh) @ wo

    def _B_ref(x, w1, b1, w2):
        h = jnp.einsum("bsd,df->bsf", x, w1) + b1
        sp = jnp.log1p(jnp.exp(-jnp.abs(h))) + jnp.where(h > 0, h, jnp.zeros_like(h))
        act = h * jnp.tanh(sp)
        return jnp.einsum("bsf,fd->bsd", act, w2)

    x = A_x
    xn = _layernorm(x, axis=-1)
    return x + _A_ref(xn, A_k_cache, A_v_cache, A_wq, A_wo) + _B_ref(xn, B_w1, B_b1, B_w2)
```

```python
import jax
import jax.numpy as jnp
from jax import lax
import jax.experimental.pallas as pl
import jax.experimental.pallas.tpu as pltpu

HQ, DH = 32, 128
_NT = (((1,), (1,)), ((), ()))
_RING = 3
_W2_CHUNKS = (1024, 512, 256)
_WO_N = 4


def _kernel(x_hbm, k_hbm, v_hbm, wq_hbm, wo_hbm, w1_hbm, b1_hbm, w2_hbm, o_ref,
            xb, b1b, kb, vb, wqb, wob, w1b, w2b, sems, small_sems):
    f32, bf16 = jnp.float32, jnp.bfloat16
    _, HKV, SK, _ = k_hbm.shape
    W = kb.shape[2]
    D, F = w1b.shape
    REP = HQ // HKV
    half_w = HQ * DH // 2
    seq = []
    seq.append(("wq0", wq_hbm.at[:, pl.ds(0, half_w)], wqb.at[:, pl.ds(0, half_w)]))
    seq.append(("wq1", wq_hbm.at[:, pl.ds(half_w, half_w)], wqb.at[:, pl.ds(half_w, half_w)]))
    for h in range(HKV):
        seq.append((f"k{h}", k_hbm.at[:, h, pl.ds(SK - W, W)], kb.at[:, h]))
        seq.append((f"v{h}", v_hbm.at[:, h, pl.ds(SK - W, W)], vb.at[:, h]))
    seq.append(("w1", w1_hbm, w1b))
    r = HQ * DH // _WO_N
    for i in range(_WO_N):
        seq.append((f"wo{i}", wo_hbm.at[pl.ds(i * r, r)], wob.at[pl.ds(i * r, r)]))
    off = 0
    for i, c in enumerate(_W2_CHUNKS):
        seq.append((f"w2{i}", w2_hbm.at[pl.ds(off, c)], w2b.at[pl.ds(off, c)]))
        off += c
    assert off == F
    n = len(seq)
    idx = {s[0]: i for i, s in enumerate(seq)}
    cps = [pltpu.make_async_copy(s[1], s[2], sems.at[i % _RING]) for i, s in enumerate(seq)]

    def wait(name):
        i = idx[name]
        cps[i].wait()
        if i + _RING < n:
            cps[i + _RING].start()

    cx = pltpu.make_async_copy(x_hbm, xb, small_sems.at[0])
    cb = pltpu.make_async_copy(b1_hbm, b1b, small_sems.at[1])
    cps[0].start()
    cx.start()
    for i in range(1, _RING):
        cps[i].start()
    cb.start()

    row = lax.broadcasted_iota(jnp.int32, (8, DH), 0)
    rowD = lax.broadcasted_iota(jnp.int32, (8, D), 0)
    cx.wait()
    x = xb[...].astype(f32)
    x8 = jnp.where(rowD < REP, jnp.broadcast_to(x[0:1], (8, D)), jnp.broadcast_to(x[1:2], (8, D)))
    mean = jnp.mean(x8, axis=-1, keepdims=True)
    xc = x8 - mean
    var = jnp.mean(xc * xc, axis=-1, keepdims=True)
    xn = (xc / jnp.sqrt(var + 1e-5)).astype(bf16)

    qs = []
    for half in range(2):
        wait(f"wq{half}")
        qf = jnp.dot(xn, wqb[:, half * half_w:(half + 1) * half_w], preferred_element_type=f32)
        for hh in range(HKV // 2):
            t = [qf[:, (hh * REP + j) * DH:(hh * REP + j + 1) * DH] for j in range(REP)]
            jj = row % REP
            qh = jnp.where(jj == 0, t[0], jnp.where(jj == 1, t[1], jnp.where(jj == 2, t[2], t[3])))
            qs.append(qh.astype(bf16))
    os_ = []
    for h in range(HKV):
        wait(f"k{h}")
        s0 = lax.dot_general(qs[h], kb[0, h], _NT, preferred_element_type=f32)
        s1 = lax.dot_general(qs[h], kb[1, h], _NT, preferred_element_type=f32)
        rowW = lax.broadcasted_iota(jnp.int32, (8, W), 0)
        s = jnp.where(rowW < REP, s0, s1) * (DH ** -0.5)
        m = jnp.max(s, axis=-1, keepdims=True)
        e = jnp.exp(s - m)
        l = jnp.sum(e, axis=-1, keepdims=True)
        p = e.astype(bf16)
        wait(f"v{h}")
        o0 = jnp.dot(p, vb[0, h], preferred_element_type=f32)
        o1 = jnp.dot(p, vb[1, h], preferred_element_type=f32)
        o = jnp.where(row < REP, o0, o1) / l
        for j in range(REP):
            os_.append(jnp.where(row % REP == j, o, 0.0).astype(bf16))
    L = jnp.concatenate(os_, axis=1)

    wait("w1")
    cb.wait()
    b1 = b1b[...].astype(f32)
    hpre = jnp.dot(xn, w1b[...], preferred_element_type=f32)
    bias = jnp.concatenate([jnp.broadcast_to(b1[j:j + 1], (8, DH)) for j in range(F // DH)], axis=1)
    hh = hpre + bias
    sp = jnp.log1p(jnp.exp(-jnp.abs(hh))) + jnp.where(hh > 0, hh, 0.0)
    act = (hh * jnp.tanh(sp)).astype(bf16)

    y = None
    for i in range(_WO_N):
        wait(f"wo{i}")
        t = jnp.dot(L[:, i * r:(i + 1) * r], wob[i * r:(i + 1) * r], preferred_element_type=f32)
        y = t if y is None else y + t
    z = None
    off = 0
    for i, c in enumerate(_W2_CHUNKS):
        wait(f"w2{i}")
        t = jnp.dot(act[:, off:off + c], w2b[off:off + c], preferred_element_type=f32)
        z = t if z is None else z + t
        off += c
    tot = y + jnp.where(rowD % REP == 0, z + x8, 0.0)
    o0 = jnp.sum(tot[0:4], axis=0, keepdims=True)
    o1 = jnp.sum(tot[4:8], axis=0, keepdims=True)
    o_ref[...] = jnp.concatenate([o0, o1], axis=0).astype(o_ref.dtype)


@jax.jit
def pallas_parallel_sum__sliding_block_cached__dense_activation_mish__decode_kernel(
    A_x: jax.Array,
    A_k_cache: jax.Array,
    A_v_cache: jax.Array,
    A_wq: jax.Array,
    A_wo: jax.Array,
    B_x: jax.Array,
    B_w1: jax.Array,
    B_b1: jax.Array,
    B_w2: jax.Array,
):
    del B_x
    B, Sq, D = A_x.shape
    _, HKV, SK, _ = A_k_cache.shape
    F = B_w1.shape[1]
    W = min(4096, max(256, SK // 4))
    bf16 = jnp.bfloat16
    out = pl.pallas_call(
        _kernel,
        in_specs=[pl.BlockSpec(memory_space=pltpu.HBM)] * 8,
        out_specs=pl.BlockSpec(memory_space=pltpu.VMEM),
        out_shape=jax.ShapeDtypeStruct((B, D), A_x.dtype),
        scratch_shapes=[
            pltpu.VMEM((B, D), bf16), pltpu.VMEM((F // DH, DH), bf16),
            pltpu.VMEM((B, HKV, W, DH), bf16), pltpu.VMEM((B, HKV, W, DH), bf16),
            pltpu.VMEM((D, HQ * DH), bf16), pltpu.VMEM((HQ * DH, D), bf16),
            pltpu.VMEM((D, F), bf16), pltpu.VMEM((F, D), bf16),
            pltpu.SemaphoreType.DMA((_RING,)), pltpu.SemaphoreType.DMA((2,)),
        ],
        compiler_params=pltpu.CompilerParams(vmem_limit_bytes=100 * 2**20),
    )(A_x.reshape(B, D), A_k_cache, A_v_cache, A_wq, A_wo, B_w1, B_b1.reshape(F // DH, DH), B_w2)
    return out.reshape(B, Sq, D)
```

```python
import jax
import jax.numpy as jnp
from jax import lax
import jax.experimental.pallas as pl
import jax.experimental.pallas.tpu as pltpu

HQ, DH = 32, 128
_NT = (((1,), (1,)), ((), ()))
_CH = 128
_W2_GROUPS = (32, 16, 8)


def _stride_order(n, stride):
    return [(i * stride) % n for i in range(n)]


def _streams(n, s):
    per = n // s
    return [sub * per + j for j in range(per) for sub in range(s)]


def _kernel(x_hbm, k_hbm, v_hbm, wq_hbm, wo_hbm, w1_hbm, b1_hbm, w2_hbm, o_ref,
            xb, b1b, kvb, wqb, wob, w1b, w2b, qb, lb, sems):
    f32, bf16 = jnp.float32, jnp.bfloat16
    _, HKV, SK, _ = k_hbm.shape
    W = kvb.shape[2]
    D, F = w1b.shape
    REP = HQ // HKV
    kv_order = [(w, c) for c in _streams(W // _CH, 2) for w in range(4)]

    def burst(pairs, sem):
        for i, (s, d) in enumerate(pairs):
            pltpu.make_async_copy(s, d, sem).start(priority=i % 2)

    def wait_all(buf, sem):
        pltpu.make_async_copy(buf, buf, sem).wait()

    def start_head(h, sem):
        burst([((k_hbm if w < 2 else v_hbm).at[w % 2, h, pl.ds(SK - W + c * _CH, _CH)],
                kvb.at[h, w, pl.ds(c * _CH, _CH)]) for w, c in kv_order], sem)

    def rows(hbm, buf, r, order):
        return [(hbm.at[pl.ds(i * r, r)], buf.at[pl.ds(i * r, r)]) for i in order]

    cx = pltpu.make_async_copy(x_hbm, xb, sems.at[2])
    cb = pltpu.make_async_copy(b1_hbm, b1b, sems.at[2])
    burst([(wq_hbm.at[pl.ds((i // 2) * 8, 8), pl.ds((i % 2) * 2048, 2048)],
            wqb.at[pl.ds((i // 2) * 8, 8), pl.ds((i % 2) * 2048, 2048)]) for i in _stride_order(128, 9)], sems.at[2])
    cx.start()
    cb.start(priority=1)
    start_head(0, sems.at[0])
    wait_all(wqb, sems.at[2])
    cx.wait()
    cb.wait()

    row = lax.broadcasted_iota(jnp.int32, (8, DH), 0)
    rowD = lax.broadcasted_iota(jnp.int32, (8, D), 0)
    x = xb[...].astype(f32)
    x8 = jnp.where(rowD < REP, jnp.broadcast_to(x[0:1], (8, D)), jnp.broadcast_to(x[1:2], (8, D)))
    mean = jnp.mean(x8, axis=-1, keepdims=True)
    xc = x8 - mean
    var = jnp.mean(xc * xc, axis=-1, keepdims=True)
    xn = (xc / jnp.sqrt(var + 1e-5)).astype(bf16)
    for h in range(HKV):
        qf = jnp.dot(xn, wqb[:, h * REP * DH:(h + 1) * REP * DH], preferred_element_type=f32)
        t = [qf[:, j * DH:(j + 1) * DH] for j in range(REP)]
        jj = row % REP
        qb[h] = jnp.where(jj == 0, t[0], jnp.where(jj == 1, t[1], jnp.where(jj == 2, t[2], t[3])))

    def head(h):
        q = qb[h].astype(bf16)
        s0 = lax.dot_general(q, kvb[h, 0], _NT, preferred_element_type=f32)
        s1 = lax.dot_general(q, kvb[h, 1], _NT, preferred_element_type=f32)
        rowW = lax.broadcasted_iota(jnp.int32, (8, W), 0)
        s = jnp.where(rowW < REP, s0, s1) * (DH ** -0.5)
        m = jnp.max(s, axis=-1, keepdims=True)
        e = jnp.exp(s - m)
        l = jnp.sum(e, axis=-1, keepdims=True)
        p = e.astype(bf16)
        o0 = jnp.dot(p, kvb[h, 2], preferred_element_type=f32)
        o1 = jnp.dot(p, kvb[h, 3], preferred_element_type=f32)
        lb[h] = jnp.where(row < REP, o0, o1) / l

    def body(h, c):
        start_head(h + 1, sems.at[(h + 1) % 2])
        wait_all(kvb.at[h], sems.at[h % 2])
        head(h)
        return c
    lax.fori_loop(0, HKV - 1, body, 0)

    burst(rows(w1_hbm, w1b, 8, _stride_order(64, 11)), sems.at[2])
    wo_pairs = rows(wo_hbm, wob, 32, _stride_order(128, 9))
    burst(wo_pairs[:64], sems.at[3])
    wait_all(kvb.at[HKV - 1], sems.at[(HKV - 1) % 2])
    head(HKV - 1)
    burst(wo_pairs[64:], sems.at[3])
    wait_all(w1b, sems.at[2])
    b1 = b1b[...].astype(f32)
    hpre = jnp.dot(xn, w1b[...], preferred_element_type=f32)
    bias = jnp.concatenate([jnp.broadcast_to(b1[j:j + 1], (8, DH)) for j in range(F // DH)], axis=1)
    hh = hpre + bias
    sp = jnp.log1p(jnp.exp(-jnp.abs(hh))) + jnp.where(hh > 0, hh, 0.0)
    act = (hh * jnp.tanh(sp)).astype(bf16)
    off = 0
    for g, n in enumerate(_W2_GROUPS):
        burst(rows(w2_hbm, w2b, 32, [off + i for i in _streams(n, 4)]), sems.at[g])
        off += n
    wait_all(wob, sems.at[3])
    L = jnp.concatenate([jnp.where(row % REP == j, lb[h], 0.0).astype(bf16)
                         for h in range(HKV) for j in range(REP)], axis=1)
    y = jnp.dot(L, wob[...], preferred_element_type=f32)
    tot = y + jnp.where(rowD % REP == 0, x8, 0.0)
    off = 0
    for g, n in enumerate(_W2_GROUPS):
        wait_all(w2b.at[pl.ds(off * 32, n * 32)], sems.at[g])
        t = jnp.dot(act[:, off * 32:(off + n) * 32], w2b[off * 32:(off + n) * 32], preferred_element_type=f32)
        tot = tot + jnp.where(rowD % REP == 0, t, 0.0)
        off += n
    o0 = jnp.sum(tot[0:4], axis=0, keepdims=True)
    o1 = jnp.sum(tot[4:8], axis=0, keepdims=True)
    o_ref[...] = jnp.concatenate([o0, o1], axis=0).astype(o_ref.dtype)


@jax.jit
def pallas_parallel_sum__sliding_block_cached__dense_activation_mish__decode_kernel(
    A_x: jax.Array,
    A_k_cache: jax.Array,
    A_v_cache: jax.Array,
    A_wq: jax.Array,
    A_wo: jax.Array,
    B_x: jax.Array,
    B_w1: jax.Array,
    B_b1: jax.Array,
    B_w2: jax.Array,
):
    del B_x
    B, Sq, D = A_x.shape
    _, HKV, SK, _ = A_k_cache.shape
    F = B_w1.shape[1]
    W = min(4096, max(256, SK // 4))
    bf16, f32 = jnp.bfloat16, jnp.float32
    out = pl.pallas_call(
        _kernel,
        in_specs=[pl.BlockSpec(memory_space=pltpu.HBM)] * 8,
        out_specs=pl.BlockSpec(memory_space=pltpu.VMEM),
        out_shape=jax.ShapeDtypeStruct((B, D), A_x.dtype),
        scratch_shapes=[
            pltpu.VMEM((B, D), bf16), pltpu.VMEM((F // DH, DH), bf16),
            pltpu.VMEM((HKV, 4, W, DH), bf16),
            pltpu.VMEM((D, HQ * DH), bf16), pltpu.VMEM((HQ * DH, D), bf16),
            pltpu.VMEM((D, F), bf16), pltpu.VMEM((F, D), bf16),
            pltpu.VMEM((HKV, 8, DH), f32), pltpu.VMEM((HKV, 8, DH), f32),
            pltpu.SemaphoreType.DMA((4,)),
        ],
        compiler_params=pltpu.CompilerParams(vmem_limit_bytes=100 * 2**20),
    )(A_x.reshape(B, D), A_k_cache, A_v_cache, A_wq, A_wo, B_w1, B_b1.reshape(F // DH, DH), B_w2)
    return out.reshape(B, Sq, D)
```

```python
import jax
import jax.numpy as jnp
from jax import lax
import jax.experimental.pallas as pl
import jax.experimental.pallas.tpu as pltpu

_HQ, _DH = 32, 128
_NT = (((1,), (1,)), ((), ()))

_KV_ROWS = 128
_WQ_ROWS, _WQ_COLS = 8, 2048
_W1_ROWS = 8
_WO_ROWS = 32
_W2_GROUPS = (40, 12, 4)
_PREFILL = 28


def _strided(n, stride):
    order = [(i * stride) % n for i in range(n)]
    assert sorted(order) == list(range(n))
    return order


def _interleaved(n, parts):
    per = n // parts
    assert per * parts == n
    return [part * per + j for j in range(per) for part in range(parts)]


def _kernel(x_hbm, k_hbm, v_hbm, wq_hbm, wo_hbm, w1_hbm, b1_hbm, w2_hbm, o_ref,
            x_buf, b1_buf, kv_buf, wq_buf, wo_buf, w1_buf, w2_buf, q_buf, att_buf, sems):
    f32, bf16 = jnp.float32, jnp.bfloat16
    B, HKV, SK, _ = k_hbm.shape
    W = kv_buf.shape[2]
    D, F = w1_buf.shape
    REP = _HQ // HKV
    assert B == 2 and B * REP == 8

    def start(copies, sem, priority=lambda i: i % 2):
        for i, (src, dst) in enumerate(copies):
            pltpu.make_async_copy(src, dst, sem).start(priority=priority(i))

    def wait(buf, sem):
        pltpu.make_async_copy(buf, buf, sem).wait()

    def row_blocks(hbm, buf, rows, order):
        return [(hbm.at[pl.ds(i * rows, rows)], buf.at[pl.ds(i * rows, rows)]) for i in order]

    def start_head(h, sem):
        start([(src.at[b, h, pl.ds(SK - W + c * _KV_ROWS, _KV_ROWS)],
                kv_buf.at[h, t * B + b, pl.ds(c * _KV_ROWS, _KV_ROWS)])
               for c in _interleaved(W // _KV_ROWS, 2)
               for t, src in enumerate((k_hbm, v_hbm))
               for b in range(B)], sem)

    per_row = wq_buf.shape[1] // _WQ_COLS
    wq_blocks = [(pl.ds(i // per_row * _WQ_ROWS, _WQ_ROWS), pl.ds(i % per_row * _WQ_COLS, _WQ_COLS))
                 for i in _strided(D // _WQ_ROWS * per_row, 9)]
    start([(wq_hbm.at[blk], wq_buf.at[blk]) for blk in wq_blocks], sems.at[2],
          lambda i: 1 if i < _PREFILL else i % 2)
    x_copy = pltpu.make_async_copy(x_hbm, x_buf, sems.at[3])
    b1_copy = pltpu.make_async_copy(b1_hbm, b1_buf, sems.at[3])
    x_copy.start(priority=0)
    b1_copy.start(priority=1)
    start_head(0, sems.at[0])
    x_copy.wait()
    b1_copy.wait()
    wait(wq_buf, sems.at[2])

    row = lax.broadcasted_iota(jnp.int32, (8, _DH), 0)
    row_d = lax.broadcasted_iota(jnp.int32, (8, D), 0)
    x = x_buf[...].astype(f32)
    x = jnp.where(row_d % B == 0, jnp.broadcast_to(x[0:1], (8, D)), jnp.broadcast_to(x[1:2], (8, D)))
    centered = x - jnp.mean(x, axis=-1, keepdims=True)
    var = jnp.mean(centered * centered, axis=-1, keepdims=True)
    xn = (centered / jnp.sqrt(var + 1e-5)).astype(bf16)

    for h in range(HKV):
        q = jnp.dot(xn, wq_buf[:, h * REP * _DH:(h + 1) * REP * _DH], preferred_element_type=f32)
        q_h = q[:, :_DH]
        for j in range(1, REP):
            q_h = jnp.where(row // B == j, q[:, j * _DH:(j + 1) * _DH], q_h)
        q_buf[h] = q_h

    def attend(h):
        q = q_buf[h].astype(bf16)
        s0 = lax.dot_general(q, kv_buf[h, 0], _NT, preferred_element_type=f32)
        s1 = lax.dot_general(q, kv_buf[h, 1], _NT, preferred_element_type=f32)
        row_w = lax.broadcasted_iota(jnp.int32, (8, W), 0)
        s = jnp.where(row_w % B == 0, s0, s1) * (_DH ** -0.5)
        e = jnp.exp(s - jnp.max(s, axis=-1, keepdims=True))
        denom = jnp.sum(e, axis=-1, keepdims=True)
        p = e.astype(bf16)
        o0 = jnp.dot(p, kv_buf[h, 2], preferred_element_type=f32)
        o1 = jnp.dot(p, kv_buf[h, 3], preferred_element_type=f32)
        att_buf[h] = jnp.where(row % B == 0, o0, o1) / denom

    def head_step(h, carry):
        start_head(h + 1, sems.at[(h + 1) % 2])
        wait(kv_buf.at[h], sems.at[h % 2])
        attend(h)
        return carry

    lax.fori_loop(0, HKV - 1, head_step, 0)

    start(row_blocks(w1_hbm, w1_buf, _W1_ROWS, _strided(D // _W1_ROWS, 11)), sems.at[2])
    wo_blocks = row_blocks(wo_hbm, wo_buf, _WO_ROWS, _strided(wo_buf.shape[0] // _WO_ROWS, 9))
    start(wo_blocks[:64], sems.at[3])
    wait(kv_buf.at[HKV - 1], sems.at[(HKV - 1) % 2])
    attend(HKV - 1)
    start(wo_blocks[64:], sems.at[3])

    wait(w1_buf, sems.at[2])
    b1 = b1_buf[...].astype(f32)
    bias = jnp.concatenate([jnp.broadcast_to(b1[j:j + 1], (8, _DH)) for j in range(F // _DH)], axis=1)
    pre = jnp.dot(xn, w1_buf[...], preferred_element_type=f32) + bias
    softplus = jnp.log1p(jnp.exp(-jnp.abs(pre))) + jnp.where(pre > 0, pre, 0.0)
    act = (pre * jnp.tanh(softplus)).astype(bf16)

    bounds = [sum(_W2_GROUPS[:g]) for g in range(len(_W2_GROUPS) + 1)]
    assert bounds[-1] * _WO_ROWS == F
    for g, n in enumerate(_W2_GROUPS):
        start(row_blocks(w2_hbm, w2_buf, _WO_ROWS, [bounds[g] + i for i in _interleaved(n, 4)]),
              sems.at[g], (lambda i: i % 2) if g == 0 else (lambda i: 1))

    wait(wo_buf, sems.at[3])
    heads = jnp.concatenate([jnp.where(row // B == j, att_buf[h], 0.0).astype(bf16)
                             for h in range(HKV) for j in range(REP)], axis=1)
    out = jnp.dot(heads, wo_buf[...], preferred_element_type=f32)
    out = out + pltpu.roll(out, 4, 0)
    out = out + pltpu.roll(out, 2, 0)
    out = out + x
    for g in range(len(_W2_GROUPS)):
        lo, hi = bounds[g] * _WO_ROWS, bounds[g + 1] * _WO_ROWS
        wait(w2_buf.at[pl.ds(lo, hi - lo)], sems.at[g])
        out = out + jnp.dot(act[:, lo:hi], w2_buf[lo:hi], preferred_element_type=f32)
    o_ref[...] = out[0:B].astype(o_ref.dtype)


@jax.jit
def pallas_parallel_sum__sliding_block_cached__dense_activation_mish__decode_kernel(
    A_x: jax.Array,
    A_k_cache: jax.Array,
    A_v_cache: jax.Array,
    A_wq: jax.Array,
    A_wo: jax.Array,
    B_x: jax.Array,
    B_w1: jax.Array,
    B_b1: jax.Array,
    B_w2: jax.Array,
):
    del B_x
    B, Sq, D = A_x.shape
    _, HKV, SK, _ = A_k_cache.shape
    F = B_w1.shape[1]
    W = min(4096, max(256, SK // 4))
    out = pl.pallas_call(
        _kernel,
        in_specs=[pl.BlockSpec(memory_space=pltpu.HBM)] * 8,
        out_specs=pl.BlockSpec(memory_space=pltpu.VMEM),
        out_shape=jax.ShapeDtypeStruct((B * Sq, D), A_x.dtype),
        scratch_shapes=[
            pltpu.VMEM((B * Sq, D), A_x.dtype),
            pltpu.VMEM((F // _DH, _DH), B_b1.dtype),
            pltpu.VMEM((HKV, 2 * B, W, _DH), A_k_cache.dtype),
            pltpu.VMEM(A_wq.shape, A_wq.dtype),
            pltpu.VMEM(A_wo.shape, A_wo.dtype),
            pltpu.VMEM(B_w1.shape, B_w1.dtype),
            pltpu.VMEM(B_w2.shape, B_w2.dtype),
            pltpu.VMEM((HKV, 8, _DH), jnp.float32),
            pltpu.VMEM((HKV, 8, _DH), jnp.float32),
            pltpu.SemaphoreType.DMA((4,)),
        ],
        compiler_params=pltpu.CompilerParams(vmem_limit_bytes=64 * 2**20),
    )(A_x.reshape(B * Sq, D), A_k_cache, A_v_cache, A_wq, A_wo, B_w1,
      B_b1.reshape(F // _DH, _DH), B_w2)
    return out.reshape(B, Sq, D)
```
